```python
import jax
import jax.numpy as jnp

def _softmax(x, axis=-1):
    return jax.nn.softmax(x, axis=axis)
def _gelu(x):
    return jax.nn.gelu(x, approximate=True)
def _silu(x):
    return jax.nn.silu(x)
def _sigmoid(x):
    return jax.nn.sigmoid(x)
def _layernorm(x, axis=-1, eps=1e-5):
    m = jnp.mean(x, axis=axis, keepdims=True)
    v = jnp.var(x, axis=axis, keepdims=True)
    return (x - m) / jnp.sqrt(v + eps)
def _scatter_add(tgt, idx, src, axis=0):
    return tgt.at[idx].add(src)
def _segment_sum(src, seg, n):
    return jax.ops.segment_sum(src, seg, n)
class _Rng:
    def __init__(self, key):
        self._k = key
    def _next(self):
        self._k, sub = jax.random.split(self._k)
        return sub
    def normal(self, shape):
        return jax.random.normal(self._next(), shape, dtype=jnp.bfloat16)
    def randint(self, lo, hi, shape):
        return jax.random.randint(self._next(), shape, lo, hi, dtype=jnp.int32)
    def uniform(self, shape, lo=0.0, hi=1.0):
        return jax.random.uniform(self._next(), shape, jnp.bfloat16, lo, hi)
    def permutation(self, n):
        return jax.random.permutation(self._next(), n)


kernel_name = 'gated_mix__gqa_block_cached__dense_activation_relu__decode'

def _fwd_setup_inputs():
    _rng = _Rng(jax.random.key(int.from_bytes(__import__("os").urandom(4), "little")))
    _w = (lambda a: (lambda t: t.astype(jnp.bfloat16) if jnp.issubdtype(t.dtype, jnp.floating) else t)(jnp.asarray(a)))
    def _A_setup():
        B, Sq, D = 2, 1, 512
        Hq, Hkv, Sk, Dh = 32, 8, 8192, 128
        assert Hq % Hkv == 0, (Hq, Hkv)
        return {
            "x": _w((lambda *s: _rng.normal(s) * 0.05)(B, Sq, D)),
            "k_cache": _w((lambda *s: _rng.normal(s) * 0.05)(B, Hkv, Sk, Dh)),
            "v_cache": _w((lambda *s: _rng.normal(s) * 0.05)(B, Hkv, Sk, Dh)),
            "wq": _w((lambda *s: _rng.normal(s) * 0.05)(D, Hq * Dh) * (D ** -0.5)),
            "wo": _w((lambda *s: _rng.normal(s) * 0.05)(Hq * Dh, D) * ((Hq * Dh) ** -0.5)),
        }
    _A_in = _A_setup()

    def _B_setup():
        B, S, D, Dff = 2, 1, 512, 1792
        return {
            "x": _w((lambda *s: _rng.normal(s) * 0.05)(B, S, D)),
            "w1": _w((lambda *s: _rng.normal(s) * 0.05)(D, Dff)),
            "w2": _w((lambda *s: _rng.normal(s) * 0.05)(Dff, D)),
        }
    _B_in = _B_setup()

    return {
        "A_x": _A_in["x"],
        "A_k_cache": _A_in["k_cache"],
        "A_v_cache": _A_in["v_cache"],
        "A_wq": _A_in["wq"],
        "A_wo": _A_in["wo"],
        "B_x": _B_in["x"],
        "B_w1": _B_in["w1"],
        "B_w2": _B_in["w2"],
        "gate_w": _w((lambda *s: _rng.normal(s) * 0.05)(512)),
    }

def _fwd_reference(A_x, A_k_cache, A_v_cache, A_wq, A_wo, B_x, B_w1, B_w2, gate_w):
    def _A_ref(x, k_cache, v_cache, wq, wo):
        B, Sq, D = x.shape
        Hq, Dh = 32, 128
        Hkv = k_cache.shape[1]
        rep = Hq // Hkv
        q = (lambda x, *d: x.transpose(*d))((x @ wq).reshape(B, Sq, Hq, Dh), 0, 2, 1, 3)
        k = jnp.repeat(k_cache, rep, axis=1)
        v = jnp.repeat(v_cache, rep, axis=1)
        scores = jnp.einsum("bhqd,bhkd->bhqk", q, k) * (Dh ** -0.5)
        p = _softmax(scores, axis=-1)
        o = jnp.einsum("bhqk,bhkd->bhqd", p, v)
        return (lambda x, *d: x.transpose(*d))(o, 0, 2, 1, 3).reshape(B, Sq, Hq * Dh) @ wo

    def _B_ref(x, w1, w2):
        h = jnp.einsum("bsd,df->bsf", x, w1)
        zero = jnp.zeros_like(h)
        h = jnp.maximum(h, zero)
        return jnp.einsum("bsf,fd->bsd", h, w2)

    x = A_x
    g = _sigmoid((x * gate_w).sum(-1, keepdims=True))
    a = _A_ref(x, A_k_cache, A_v_cache, A_wq, A_wo)
    b = _B_ref(x, B_w1, B_w2)
    return g * a + (1 - g) * b


def setup_inputs():
    _inp = _fwd_setup_inputs()
    _gk = jax.random.fold_in(jax.random.key(int.from_bytes(__import__("os").urandom(4), "little")), 2**31 - 1)
    _shapes = [[2, 1, 512]]
    _dtypes = ['bfloat16']
    _gks = jax.random.split(_gk, len(_shapes))
    _gs = [jax.random.normal(k, s, dtype=jnp.dtype(d)) * 0.05 for k, s, d in zip(_gks, _shapes, _dtypes)]
    _inp["grad_out"] = _gs[0]
    return _inp

def reference(A_x, A_k_cache, A_v_cache, A_wq, A_wo, B_w1, B_w2, gate_w, B_x, grad_out):
    _const = dict(B_x=B_x)
    def _f(*_d):
        return _fwd_reference(**{'A_x': _d[0], 'A_k_cache': _d[1], 'A_v_cache': _d[2], 'A_wq': _d[3], 'A_wo': _d[4], 'B_w1': _d[5], 'B_w2': _d[6], 'gate_w': _d[7], **_const})
    _out, _vjp = jax.vjp(_f, A_x, A_k_cache, A_v_cache, A_wq, A_wo, B_w1, B_w2, gate_w)
    _grads = _vjp(grad_out)
    _out0 = jnp.asarray(_out)
    return (_out0, *[jnp.asarray(_g) for _g in _grads])
```

```python
import jax
import jax.numpy as jnp
from jax import lax
import jax.experimental.pallas as pl
import jax.experimental.pallas.tpu as pltpu

F32 = jnp.float32
BF16 = jnp.bfloat16

B, D, HQ, HKV, SK, DH, DFF = 2, 512, 32, 8, 8192, 128, 1792
REP = HQ // HKV
NU = B * HKV
STREAM = 4096
NS = NU * SK // STREAM
WIN = 8
NW = NS // WIN
GU = NU // NW
CH = 2048
NC = SK // CH

NN = (((1,), (0,)), ((), ()))
NT = (((1,), (1,)), ((), ()))
TN = (((0,), (0,)), ((), ()))


def _dot(a, b, dims):
    return lax.dot_general(a, b, dims, preferred_element_type=F32)


def make(piece=64, last_pieces=24, compute=True, **cparams):
    NP = STREAM // piece
    PC = CH // piece
    scale = DH ** -0.5

    def kernel(x_hbm, k_hbm, v_hbm, wq_hbm, wo_hbm, w1_hbm, w2_hbm, gw_hbm, go_hbm,
               out_hbm, dx_hbm, dk_hbm, dv_hbm, dwq_hbm, dwo_hbm, dw1_hbm, dw2_hbm, dgw_hbm,
               kbuf, vbuf, wq, wo, w1, w2, dwq, dwo, dw1, dw2,
               x_v, gw_v, go_v, out_v, dx_v, dgw_v,
               qq, dd, pd, od, s_scr, dp_scr, sem):
        copy = pltpu.make_async_copy

        def rd_weights():
            return [copy(wq_hbm, wq, sem.at[0]), copy(x_hbm, x_v, sem.at[0]), copy(gw_hbm, gw_v, sem.at[0]),
                    copy(go_hbm, go_v, sem.at[0]), copy(wo_hbm, wo, sem.at[0]),
                    copy(w1_hbm, w1, sem.at[0]), copy(w2_hbm, w2, sem.at[0])]

        def rd_group(g):
            s = sem.at[(g + 1) % 3]
            sl = pl.ds(g * WIN, WIN)
            cs = [copy(k_hbm.at[sl], kbuf.at[sl], s)]
            if g < NW - 1 or not last_pieces:
                return cs + [copy(v_hbm.at[sl], vbuf.at[sl], s)]
            sl = pl.ds(g * WIN, WIN - 1)
            head = (NS - 1, pl.ds(0, NP - last_pieces))
            return cs + [copy(v_hbm.at[sl], vbuf.at[sl], s), copy(v_hbm.at[head], vbuf.at[head], s)]

        def rd_tail():
            if not last_pieces:
                return []
            tail = (NS - 1, pl.ds(NP - last_pieces, last_pieces))
            return [copy(v_hbm.at[tail], vbuf.at[tail], sem.at[(NW + 1) % 3])]

        def start(cs):
            for c in cs:
                c.start()

        def wait(cs):
            for c in cs:
                c.wait()

        start(rd_weights())
        start(rd_group(0))
        start(rd_group(1))

        wsem = sem.at[0]

        def start_kv_writes(src, dst, w):
            sl = pl.ds(w * WIN, WIN)

            @pl.loop(0, NP)
            def _(j):
                copy(src.at[sl, j], dst.at[sl, j], wsem).start()

        def start_qo_writes():
            @pl.loop(0, 16)
            def _(i):
                rows = pl.ds(pl.multiple_of(i * 8, 8), 8)
                for c in range(4):
                    cols = pl.ds(c * 1024, 1024)
                    copy(dwq.at[:, rows, cols], dwq_hbm.at[:, rows, cols], wsem).start()
                    copy(dwo.at[:, i * 4 + c], dwo_hbm.at[:, i * 4 + c], wsem).start()

        def start_mlp_writes():
            @pl.loop(0, 16)
            def _(i):
                rows = pl.ds(pl.multiple_of(i * 8, 8), 8)
                for c in range(2):
                    cols = pl.ds(c * 896, 896)
                    copy(dw1.at[:, rows, cols], dw1_hbm.at[:, rows, cols], wsem).start()

                    @pl.when(i < 14)
                    def _():
                        copy(dw2.at[:, i * 2 + c], dw2_hbm.at[:, i * 2 + c], wsem).start()

        def wr_small():
            return [copy(out_v, out_hbm, wsem), copy(dx_v, dx_hbm, wsem), copy(dgw_v, dgw_hbm, wsem)]

        wait(rd_weights())
        start(rd_group(2))
        row8 = lax.broadcasted_iota(jnp.int32, (8, D), 0)

        def rows2(ref):
            t = ref[...].astype(F32)
            r0 = jnp.broadcast_to(t[0:1], (8, D))
            r1 = jnp.broadcast_to(t[1:2], (8, D))
            return jnp.where(row8 == 0, r0, jnp.where(row8 == 1, r1, 0.0))

        x = rows2(x_v)
        go = rows2(go_v)
        gw = gw_v[...].astype(F32).reshape(1, D)
        z = jnp.sum(x * gw, axis=1, keepdims=True)
        g = 1.0 / (1.0 + jnp.exp(-z))
        da = (g * go).astype(BF16)
        db = ((1.0 - g) * go).astype(BF16)
        xb = x.astype(BF16)

        row = lax.broadcasted_iota(jnp.int32, (8, DH), 0)

        def heads_to_rows(t, b):
            acc = jnp.broadcast_to(t[b:b + 1, 0:DH], (8, DH))
            for h in range(1, REP):
                r = jnp.broadcast_to(t[b:b + 1, h * DH:(h + 1) * DH], (8, DH))
                acc = jnp.where(row % REP == h, r, acc)
            return acc

        if compute:
            for kv in range(HKV):
                t = _dot(xb, wq[:, kv * 512:(kv + 1) * 512], NN)
                for b in range(B):
                    qq[b * HKV + kv] = heads_to_rows(t, b)
            for kv in range(HKV):
                t = _dot(da, wo[kv * 512:(kv + 1) * 512, :], NT)
                for b in range(B):
                    dd[b * HKV + kv] = heads_to_rows(t, b)

            h = _dot(xb, w1[...], NN).astype(BF16).astype(F32)
            hr = jnp.maximum(h, 0.0).astype(BF16)
            bout = _dot(hr, w2[...], NN)
            dhr = _dot(db, w2[...], NT)
            slope = jnp.where(h > 0.0, 1.0, jnp.where(h == 0.0, 0.5, 0.0))
            dh = (dhr * slope).astype(BF16)
            dx_b = _dot(dh, w1[...], NT)
            for c in range(4):
                dw1[c] = _dot(xb[:, c * 128:(c + 1) * 128], dh, TN).astype(BF16)
            for c in range(7):
                r = _dot(hr[:, c * 256:(c + 1) * 256], db, TN).astype(BF16)
                for i in range(16):
                    gi = c * 16 + i
                    dw2[gi // 28, gi % 28] = r[i * 16:(i + 1) * 16]

        rowc = lax.broadcasted_iota(jnp.int32, (8, CH), 0)

        def chunk(u, c):
            return (2 * u + c // 2, pl.ds((c % 2) * PC, PC))

        def phase1(u):
            q = qq[u].astype(BF16)
            do = dd[u].astype(BF16)
            m = None
            for c in range(NC):
                s = _dot(q, kbuf[chunk(u, c)].reshape(CH, DH), NT) * scale
                s_scr[c] = s
                mc = jnp.max(s, axis=1, keepdims=True)
                m = mc if m is None else jnp.maximum(m, mc)
            l = 0.0
            t = 0.0
            for c in range(NC):
                dp = _dot(do, vbuf[chunk(u, c)].reshape(CH, DH), NT)
                dp_scr[c] = dp
                e = jnp.exp(s_scr[c] - m)
                s_scr[c] = e
                l = l + jnp.sum(e, axis=1, keepdims=True)
                t = t + jnp.sum(e * dp, axis=1, keepdims=True)
            rl = 1.0 / l
            delta = t * rl
            o = jnp.zeros((8, DH), F32)
            dq = jnp.zeros((8, DH), F32)
            for c in range(NC):
                p = s_scr[c] * rl
                ds = p * (dp_scr[c] - delta) * scale
                t2 = jnp.where(rowc < REP, p, ds)
                pd[u * NC + c] = t2
                t2 = t2.astype(BF16)
                o = o + _dot(t2, vbuf[chunk(u, c)].reshape(CH, DH), NN)
                dq = dq + _dot(t2, kbuf[chunk(u, c)].reshape(CH, DH), NN)
            od[u] = jnp.where(row < REP, o, dq)

        def phase2(u):
            wv = jnp.where(row < REP, dd[u], 0.0)
            wk = jnp.where(row < REP, 0.0, qq[u])
            w = jnp.concatenate([wv, wk], axis=1).astype(BF16)

            @pl.loop(0, NC)
            def _(c):
                for i in range(2):
                    n = CH // 2
                    r = _dot(pd[u * NC + c, :, i * n:(i + 1) * n].astype(BF16), w, TN).astype(BF16)
                    idx = (2 * u + c // 2, pl.ds((c % 2) * PC + i * (PC // 2), PC // 2))
                    vbuf[idx] = r[:, :DH].reshape(PC // 2, piece, DH)
                    kbuf[idx] = r[:, DH:].reshape(PC // 2, piece, DH)

        @pl.loop(0, NU + GU)
        def _(t):
            @pl.when(t == 0)
            def _():
                wait(rd_group(0))
                start(rd_group(3))

            @pl.when(t == GU)
            def _():
                wait(rd_group(1))
                start(rd_tail())

            @pl.when(t == 2 * GU)
            def _():
                wait(rd_group(2))

            @pl.when(t == 3 * GU)
            def _():
                wait(rd_group(3))
                start_mlp_writes()
                wait(rd_tail())

            @pl.when((t == 12) | (t == 14) | (t == 16))
            def _():
                start_kv_writes(vbuf, dv_hbm, (t - 12) // 2)

            @pl.when((t == 13) | (t == 15) | (t == 18))
            def _():
                start_kv_writes(kbuf, dk_hbm, (t - 13) // 2)

            if compute:
                @pl.when(t < NU)
                def _():
                    phase1(t)

                @pl.when((t < 2 * GU) | (t >= 3 * GU))
                def _():
                    phase2(jnp.where(t < 2 * GU, t, t - GU))

        start_kv_writes(vbuf, dv_hbm, NW - 1)

        if compute:
            def rows_to_heads(kv, off):
                parts = []
                for hh in range(REP):
                    r0 = jnp.broadcast_to(od[kv, off + hh:off + hh + 1, :], (8, DH))
                    r1 = jnp.broadcast_to(od[HKV + kv, off + hh:off + hh + 1, :], (8, DH))
                    parts.append(jnp.where(row == 0, r0, jnp.where(row == 1, r1, 0.0)))
                return jnp.concatenate(parts, axis=1).astype(BF16)

            a = jnp.zeros((8, D), F32)
            dx_a = jnp.zeros((8, D), F32)
            for kv in range(HKV):
                o_kv = rows_to_heads(kv, 0)
                dq_kv = rows_to_heads(kv, REP)
                a = a + _dot(o_kv, wo[kv * 512:(kv + 1) * 512, :], NN)
                dx_a = dx_a + _dot(dq_kv, wq[:, kv * 512:(kv + 1) * 512], NT)
                r = _dot(o_kv, da, TN).astype(BF16)
                r2 = _dot(xb, dq_kv, TN).astype(BF16)
                dwo[kv // 2, (kv % 2) * 32:(kv % 2 + 1) * 32] = r.reshape(32, 16, D)
                dwq[:, :, kv * 512:(kv + 1) * 512] = r2.reshape(4, 128, 512)
            out = g * a + (1.0 - g) * bout
            dg = jnp.sum(go * (a - bout), axis=1, keepdims=True)
            dz = dg * g * (1.0 - g)
            dx = dx_a + dx_b + dz * gw
            dgw = jnp.sum(dz * x, axis=0, keepdims=True)
            out_v[...] = out[0:B].astype(BF16)
            dx_v[...] = dx[0:B].astype(BF16)
            dgw_v[...] = dgw.astype(BF16).reshape(D)

        start(wr_small())
        start_qo_writes()
        start_kv_writes(kbuf, dk_hbm, NW - 1)

        wait(wr_small())
        wait([copy(dw1, dw1_hbm, wsem), copy(dw2, dw2_hbm, wsem), copy(dwq, dwq_hbm, wsem),
              copy(dwo, dwo_hbm, wsem), copy(vbuf, dv_hbm, wsem), copy(kbuf, dk_hbm, wsem)])

    hbm = pl.BlockSpec(memory_space=pltpu.HBM)
    kv_shape = (NS, NP, piece, DH)
    dwq_shape = (4, D // 4, HQ * DH)
    dwo_shape = (4, 64, 16, D)
    dw1_shape = (4, D // 4, DFF)
    dw2_shape = (4, 28, 16, D)
    sds = jax.ShapeDtypeStruct

    @jax.jit
    def fn(A_x, A_k_cache, A_v_cache, A_wq, A_wo, B_x, B_w1, B_w2, gate_w, grad_out):
        del B_x
        outs = pl.pallas_call(
            kernel,
            out_shape=[sds((B, D), BF16), sds((B, D), BF16), sds(kv_shape, BF16), sds(kv_shape, BF16),
                       sds(dwq_shape, BF16), sds(dwo_shape, BF16), sds(dw1_shape, BF16), sds(dw2_shape, BF16),
                       sds((D,), BF16)],
            in_specs=[hbm] * 9,
            out_specs=[hbm] * 9,
            scratch_shapes=[
                pltpu.VMEM(kv_shape, BF16), pltpu.VMEM(kv_shape, BF16),
                pltpu.VMEM((D, HQ * DH), BF16), pltpu.VMEM((HQ * DH, D), BF16),
                pltpu.VMEM((D, DFF), BF16), pltpu.VMEM((DFF, D), BF16),
                pltpu.VMEM(dwq_shape, BF16), pltpu.VMEM(dwo_shape, BF16),
                pltpu.VMEM(dw1_shape, BF16), pltpu.VMEM(dw2_shape, BF16),
                pltpu.VMEM((B, D), BF16), pltpu.VMEM((D,), BF16), pltpu.VMEM((B, D), BF16),
                pltpu.VMEM((B, D), BF16), pltpu.VMEM((B, D), BF16), pltpu.VMEM((D,), BF16),
                pltpu.VMEM((NU, 8, DH), F32), pltpu.VMEM((NU, 8, DH), F32),
                pltpu.VMEM((NU * NC, 8, CH), F32), pltpu.VMEM((NU, 8, DH), F32),
                pltpu.VMEM((NC, 8, CH), F32), pltpu.VMEM((NC, 8, CH), F32),
                pltpu.SemaphoreType.DMA((3,)),
            ],
            compiler_params=pltpu.CompilerParams(vmem_limit_bytes=112 * 1024 * 1024, **cparams),
        )(A_x.reshape(B, D), A_k_cache.reshape(kv_shape), A_v_cache.reshape(kv_shape), A_wq, A_wo, B_w1, B_w2,
          gate_w, grad_out.reshape(B, D))
        out, dx, dk, dv, gwq, gwo, gw1, gw2, ggw = outs
        return (out.reshape(A_x.shape), dx.reshape(A_x.shape), dk.reshape(A_k_cache.shape),
                dv.reshape(A_v_cache.shape), gwq.reshape(A_wq.shape), gwo.reshape(A_wo.shape),
                gw1.reshape(B_w1.shape), gw2.reshape(B_w2.shape), ggw)

    return fn


pallas_gated_mix__gqa_block_cached__dense_activation_relu__decode_kernel = make()
```

```python
import jax
import jax.numpy as jnp
from jax import lax
import jax.experimental.pallas as pl
import jax.experimental.pallas.tpu as pltpu

F32 = jnp.float32
BF16 = jnp.bfloat16

B, D, HQ, HKV, SK, DH, DFF = 2, 512, 32, 8, 8192, 128, 1792
REP = HQ // HKV
GW = REP * DH
NU = B * HKV
ROWS = 8

CH = 2048
NC = SK // CH
STREAM = 4096
NS = NU * SK // STREAM
GROUP = 4
NG = NU // GROUP
TAIL = 1408
PIECE = 72
WINDOWS = (7, 7, 6, 6, 6)

NN = (((1,), (0,)), ((), ()))
NT = (((1,), (1,)), ((), ()))
TN = (((0,), (0,)), ((), ()))


def _dot(a, b, dims):
    return lax.dot_general(a, b, dims, preferred_element_type=F32)


def _start(copies):
    for c in copies:
        c.start()


def _wait(copies):
    for c in copies:
        c.wait()


def _kernel(
    x_hbm, k_hbm, v_hbm, wq_hbm, wo_hbm, w1_hbm, w2_hbm, gw_hbm, go_hbm,
    out_hbm, dx_hbm, dk_hbm, dv_hbm, dwq_hbm, dwo_hbm, dw1_hbm, dw2_hbm, dgw_hbm,
    kbuf, vbuf, wq, wo, w1, w2, dwq, dwo, dw1, dw2,
    x_v, gw_v, go_v, out_v, dx_v, dgw_v,
    q_scr, do_scr, pds_scr, odq_scr, s_scr, dp_scr, sems,
):
    copy = pltpu.make_async_copy

    def read_batch(i):
        sem = sems.at[i % 2]
        if i == 0:
            return [copy(wq_hbm, wq, sem), copy(x_hbm, x_v, sem), copy(gw_hbm, gw_v, sem),
                    copy(go_hbm, go_v, sem), copy(wo_hbm, wo, sem),
                    copy(w1_hbm, w1, sem), copy(w2_hbm, w2, sem)]
        if i == NG + 1:
            tail = (NS - 1, pl.ds(STREAM - TAIL, TAIL))
            return [copy(v_hbm.at[tail], vbuf.at[tail], sem)]
        n = NS // NG
        group = pl.ds((i - 1) * n, n)
        copies = [copy(k_hbm.at[group], kbuf.at[group], sem)]
        if i < NG:
            return copies + [copy(v_hbm.at[group], vbuf.at[group], sem)]
        group = pl.ds((i - 1) * n, n - 1)
        head = (NS - 1, pl.ds(0, STREAM - TAIL))
        return copies + [copy(v_hbm.at[group], vbuf.at[group], sem),
                         copy(v_hbm.at[head], vbuf.at[head], sem)]

    def finish_read_batch(i):
        _wait(read_batch(i))
        if i + 2 <= NG + 1:
            _start(read_batch(i + 2))

    wsem = sems.at[NG % 2]

    def start_cache_writes(window, src, dst):
        streams = pl.ds(sum(WINDOWS[:window]), WINDOWS[window])

        @pl.loop(0, STREAM // PIECE)
        def _(j):
            rows = pl.ds(pl.multiple_of(j * PIECE, 8), PIECE)
            copy(src.at[streams, rows], dst.at[streams, rows], wsem).start()

        if STREAM % PIECE:
            rows = pl.ds(STREAM - STREAM % PIECE, STREAM % PIECE)
            copy(src.at[streams, rows], dst.at[streams, rows], wsem).start()

    def start_mlp_writes():
        @pl.loop(0, 16)
        def _(i):
            rows = pl.ds(pl.multiple_of(i * 8, 8), 8)
            for c in range(2):
                cols = pl.ds(c * (DFF // 2), DFF // 2)
                copy(dw1.at[:, rows, cols], dw1_hbm.at[:, rows, cols], wsem).start()

                @pl.when(i < 14)
                def _():
                    copy(dw2.at[:, 2 * i + c], dw2_hbm.at[:, 2 * i + c], wsem).start()

    def start_proj_writes():
        @pl.loop(0, 16)
        def _(i):
            rows = pl.ds(pl.multiple_of(i * 8, 8), 8)
            for c in range(4):
                cols = pl.ds(c * 1024, 1024)
                copy(dwq.at[:, rows, cols], dwq_hbm.at[:, rows, cols], wsem).start()
                copy(dwo.at[:, 4 * i + c], dwo_hbm.at[:, 4 * i + c], wsem).start()

    def small_writes():
        return [copy(out_v, out_hbm, wsem), copy(dx_v, dx_hbm, wsem), copy(dgw_v, dgw_hbm, wsem)]

    _start(read_batch(0))
    _start(read_batch(1))
    finish_read_batch(0)

    def two_rows(r0, r1):
        shape = (ROWS, r0.shape[1])
        i = lax.broadcasted_iota(jnp.int32, shape, 0)
        return jnp.where(i == 0, jnp.broadcast_to(r0, shape),
                         jnp.where(i == 1, jnp.broadcast_to(r1, shape), 0.0))

    x = x_v[...].astype(F32)
    x = two_rows(x[0:1], x[1:2])
    go = go_v[...].astype(F32)
    go = two_rows(go[0:1], go[1:2])
    gw = gw_v[...].astype(F32).reshape(1, D)
    g = jax.nn.sigmoid(jnp.sum(x * gw, axis=1, keepdims=True))
    xb = x.astype(BF16)
    da = (g * go).astype(BF16)
    db = ((1.0 - g) * go).astype(BF16)

    row = lax.broadcasted_iota(jnp.int32, (ROWS, DH), 0)

    def heads_to_rows(t, b):
        tile = jnp.broadcast_to(t[b:b + 1, :DH], (ROWS, DH))
        for h in range(1, REP):
            head = jnp.broadcast_to(t[b:b + 1, h * DH:(h + 1) * DH], (ROWS, DH))
            tile = jnp.where(row % REP == h, head, tile)
        return tile

    for kv in range(HKV):
        q = _dot(xb, wq[:, kv * GW:(kv + 1) * GW], NN)
        do = _dot(da, wo[kv * GW:(kv + 1) * GW, :], NT)
        for b in range(B):
            q_scr[b * HKV + kv] = heads_to_rows(q, b)
            do_scr[b * HKV + kv] = heads_to_rows(do, b)

    h = _dot(xb, w1[...], NN).astype(BF16).astype(F32)
    act = jnp.maximum(h, 0.0).astype(BF16)
    mlp_out = _dot(act, w2[...], NN)
    slope = jnp.where(h > 0.0, 1.0, jnp.where(h == 0.0, 0.5, 0.0))
    dh = (_dot(db, w2[...], NT) * slope).astype(BF16)
    dx_mlp = _dot(dh, w1[...], NT)
    for c in range(4):
        dw1[c] = _dot(xb[:, c * 128:(c + 1) * 128], dh, TN).astype(BF16)
    for c in range(DFF // 256):
        r = _dot(act[:, c * 256:(c + 1) * 256], db, TN).astype(BF16)
        for i in range(16):
            dw2[divmod(c * 16 + i, dw2.shape[1])] = r[i * 16:(i + 1) * 16]

    scale = DH ** -0.5
    chunk_row = lax.broadcasted_iota(jnp.int32, (ROWS, CH), 0)

    def chunk(u, c):
        return 2 * u + c // 2, pl.ds((c % 2) * CH, CH)

    def attend(u):
        q = q_scr[u].astype(BF16)
        do = do_scr[u].astype(BF16)
        m = None
        for c in range(NC):
            s = _dot(q, kbuf[chunk(u, c)], NT) * scale
            s_scr[c] = s
            mc = jnp.max(s, axis=1, keepdims=True)
            m = mc if m is None else jnp.maximum(m, mc)
        denom = 0.0
        e_dp = 0.0
        for c in range(NC):
            dp = _dot(do, vbuf[chunk(u, c)], NT)
            dp_scr[c] = dp
            e = jnp.exp(s_scr[c] - m)
            s_scr[c] = e
            denom = denom + jnp.sum(e, axis=1, keepdims=True)
            e_dp = e_dp + jnp.sum(e * dp, axis=1, keepdims=True)
        inv = 1.0 / denom
        delta = e_dp * inv
        o = jnp.zeros((ROWS, DH), F32)
        dq = jnp.zeros((ROWS, DH), F32)
        for c in range(NC):
            p = s_scr[c] * inv
            ds = p * (dp_scr[c] - delta) * scale
            pds = jnp.where(chunk_row < REP, p, ds)
            pds_scr[u * NC + c] = pds
            pds = pds.astype(BF16)
            o = o + _dot(pds, vbuf[chunk(u, c)], NN)
            dq = dq + _dot(pds, kbuf[chunk(u, c)], NN)
        odq_scr[u] = jnp.where(row < REP, o, dq)

    def cache_grads(u):
        w = jnp.concatenate([jnp.where(row < REP, do_scr[u], 0.0),
                             jnp.where(row < REP, 0.0, q_scr[u])], axis=1).astype(BF16)
        n = CH // 2

        @pl.loop(0, NC)
        def _(c):
            for i in range(2):
                pds = pds_scr[u * NC + c, :, i * n:(i + 1) * n].astype(BF16)
                r = _dot(pds, w, TN).astype(BF16)
                rows = 2 * u + c // 2, pl.ds(pl.multiple_of((c % 2) * CH + i * n, n), n)
                vbuf[rows] = r[:, :DH]
                kbuf[rows] = r[:, DH:]

    first_write = (NG - 1) * GROUP

    @pl.loop(0, NU + GROUP)
    def _(t):
        for i in range(1, NG + 1):
            @pl.when(t == (i - 1) * GROUP)
            def _():
                finish_read_batch(i)
                if i == NG:
                    start_mlp_writes()
                    finish_read_batch(NG + 1)

        for i in range(2 * (len(WINDOWS) - 1)):
            @pl.when(t == first_write + i)
            def _():
                start_cache_writes(i // 2, *((kbuf, dk_hbm) if i % 2 else (vbuf, dv_hbm)))

        @pl.when(t < NU)
        def _():
            attend(t)

        @pl.when((t < first_write - GROUP) | (t >= first_write))
        def _():
            cache_grads(jnp.where(t < first_write, t, t - GROUP))

    def rows_to_heads(kv, first):
        return jnp.concatenate(
            [two_rows(odq_scr[kv, r:r + 1, :], odq_scr[HKV + kv, r:r + 1, :])
             for r in range(first, first + REP)], axis=1).astype(BF16)

    attn_out = jnp.zeros((ROWS, D), F32)
    dx_attn = jnp.zeros((ROWS, D), F32)
    for kv in range(HKV):
        if kv == 0:
            start_cache_writes(len(WINDOWS) - 1, vbuf, dv_hbm)
        if kv == HKV // 2:
            start_cache_writes(len(WINDOWS) - 1, kbuf, dk_hbm)
        o = rows_to_heads(kv, 0)
        dq = rows_to_heads(kv, REP)
        attn_out = attn_out + _dot(o, wo[kv * GW:(kv + 1) * GW, :], NN)
        dx_attn = dx_attn + _dot(dq, wq[:, kv * GW:(kv + 1) * GW], NT)
        dwo[kv // 2, (kv % 2) * 32:(kv % 2 + 1) * 32] = (
            _dot(o, da, TN).astype(BF16).reshape(32, 16, D))
        dwq[:, :, kv * GW:(kv + 1) * GW] = _dot(xb, dq, TN).astype(BF16).reshape(4, D // 4, GW)

    dz = jnp.sum(go * (attn_out - mlp_out), axis=1, keepdims=True) * g * (1.0 - g)
    out_v[...] = (g * attn_out + (1.0 - g) * mlp_out)[:B].astype(BF16)
    dx_v[...] = (dx_attn + dx_mlp + dz * gw)[:B].astype(BF16)
    dgw_v[...] = jnp.sum(dz * x, axis=0, keepdims=True).astype(BF16).reshape(D)
    _start(small_writes())
    start_proj_writes()

    _wait(small_writes())
    _wait([copy(dw1, dw1_hbm, wsem), copy(dw2, dw2_hbm, wsem), copy(dwq, dwq_hbm, wsem),
           copy(dwo, dwo_hbm, wsem), copy(vbuf, dv_hbm, wsem), copy(kbuf, dk_hbm, wsem)])


@jax.jit
def pallas_gated_mix__gqa_block_cached__dense_activation_relu__decode_kernel(
    A_x: jax.Array,
    A_k_cache: jax.Array,
    A_v_cache: jax.Array,
    A_wq: jax.Array,
    A_wo: jax.Array,
    B_x: jax.Array,
    B_w1: jax.Array,
    B_w2: jax.Array,
    gate_w: jax.Array,
    grad_out: jax.Array,
):
    del B_x

    cache = (NS, STREAM, DH)
    dwq, dwo = (4, D // 4, HQ * DH), (4, HQ * DH // 64, 16, D)
    dw1, dw2 = (4, D // 4, DFF), (4, DFF // 64, 16, D)
    out_shapes = [(B, D), (B, D), cache, cache, dwq, dwo, dw1, dw2, (D,)]
    hbm = pl.BlockSpec(memory_space=pltpu.HBM)

    outs = pl.pallas_call(
        _kernel,
        out_shape=[jax.ShapeDtypeStruct(s, BF16) for s in out_shapes],
        in_specs=[hbm] * 9,
        out_specs=[hbm] * 9,
        scratch_shapes=[
            *[pltpu.VMEM(s, BF16) for s in (
                cache, cache, A_wq.shape, A_wo.shape, B_w1.shape, B_w2.shape, dwq, dwo, dw1, dw2,
                (B, D), (D,), (B, D), (B, D), (B, D), (D,))],
            *[pltpu.VMEM(s, F32) for s in (
                (NU, ROWS, DH), (NU, ROWS, DH), (NU * NC, ROWS, CH), (NU, ROWS, DH),
                (NC, ROWS, CH), (NC, ROWS, CH))],
            pltpu.SemaphoreType.DMA((2,)),
        ],
        compiler_params=pltpu.CompilerParams(vmem_limit_bytes=110 * 1024 * 1024),
    )(A_x.reshape(B, D), A_k_cache.reshape(cache), A_v_cache.reshape(cache), A_wq, A_wo,
      B_w1, B_w2, gate_w, grad_out.reshape(B, D))

    like = (A_x, A_x, A_k_cache, A_v_cache, A_wq, A_wo, B_w1, B_w2, gate_w)
    return tuple(o.reshape(a.shape) for o, a in zip(outs, like))
```
